```python
import os as _os
_os.environ.setdefault("JAX_PLATFORMS", "cpu")
import jax
import jax.numpy as jnp

def _softmax(x, axis=-1):
    return jax.nn.softmax(x, axis=axis)
def _gelu(x):
    return jax.nn.gelu(x, approximate=True)
def _silu(x):
    return jax.nn.silu(x)
def _sigmoid(x):
    return jax.nn.sigmoid(x)
def _layernorm(x, axis=-1, eps=1e-5):
    m = jnp.mean(x, axis=axis, keepdims=True)
    v = jnp.var(x, axis=axis, keepdims=True)
    return (x - m) / jnp.sqrt(v + eps)
def _scatter_add(tgt, idx, src, axis=0):
    return tgt.at[idx].add(src)
def _segment_sum(src, seg, n):
    return jax.ops.segment_sum(src, seg, n)
class _Rng:
    def __init__(self, key):
        self._k = key
    def _next(self):
        self._k, sub = jax.random.split(self._k)
        return sub
    def normal(self, shape):
        return jax.random.normal(self._next(), shape, dtype=jnp.bfloat16)
    def randint(self, lo, hi, shape):
        return jax.random.randint(self._next(), shape, lo, hi, dtype=jnp.int32)
    def uniform(self, shape, lo=0.0, hi=1.0):
        return jax.random.uniform(self._next(), shape, jnp.bfloat16, lo, hi)
    def permutation(self, n):
        return jax.random.permutation(self._next(), n)


kernel_name = 'interleave_layers__mha_block__dense_activation_mish__prompt'

def setup_inputs():
    _rng = _Rng(jax.random.key(int.from_bytes(__import__("os").urandom(4), "little")))
    _w = (lambda a: (lambda t: t.astype(jnp.bfloat16) if jnp.issubdtype(t.dtype, jnp.floating) else t)(jnp.asarray(a)))
    def _A_setup():
        B, S, D, H = 1, 2048, 512, 32
        return {
            "x": _w((lambda *s: _rng.normal(s) * 0.05)(B, S, D)),
            "wqkv": _w((lambda *s: _rng.normal(s) * 0.05)(D, 3 * D)),
            "wo": _w((lambda *s: _rng.normal(s) * 0.05)(D, D)),
        }
    _A_in = _A_setup()

    def _B_setup():
        B, S, D, F = 1, 2048, 512, 1792
        return {
            "x": _w((lambda *s: _rng.normal(s) * 0.05)(B, S, D)),
            "w1": _w((lambda *s: _rng.normal(s) * 0.4)(D, F) * (D ** -0.5)),
            "b1": _w((lambda *s: _rng.normal(s) * 0.4)(F)),
            "w2": _w((lambda *s: _rng.normal(s) * 0.4)(F, D) * (F ** -0.5)),
        }
    _B_in = _B_setup()

    return {
        "A_x": _A_in["x"],
        "A_wqkv": _A_in["wqkv"],
        "A_wo": _A_in["wo"],
        "B_x": _B_in["x"],
        "B_w1": _B_in["w1"],
        "B_b1": _B_in["b1"],
        "B_w2": _B_in["w2"],
    }

def reference(A_x, A_wqkv, A_wo, B_x, B_w1, B_b1, B_w2):
    def _A_ref(x, wqkv, wo):
        B, S, D = x.shape
        H = 32
        Dh = D // H
        qkv = (lambda x, *d: x.transpose(*d))((x @ wqkv).reshape(B, S, 3, H, Dh), 2, 0, 3, 1, 4)
        q, k, v = qkv[0], qkv[1], qkv[2]
        scores = jnp.einsum("bhqd,bhkd->bhqk", q, k) * (Dh ** -0.5)
        p = _softmax(scores, axis=-1)
        o = jnp.einsum("bhqk,bhkd->bhqd", p, v)
        return (lambda x, *d: x.transpose(*d))(o, 0, 2, 1, 3).reshape(B, S, D) @ wo

    def _B_ref(x, w1, b1, w2):
        h = jnp.einsum("bsd,df->bsf", x, w1) + b1
        sp = jnp.log1p(jnp.exp(-jnp.abs(h))) + jnp.where(h > 0, h, jnp.zeros_like(h))
        act = h * jnp.tanh(sp)
        return jnp.einsum("bsf,fd->bsd", act, w2)

    x = A_x
    x = x + _A_ref(_layernorm(x, axis=-1), A_wqkv, A_wo)
    x = x + _B_ref(_layernorm(x, axis=-1), B_w1, B_b1, B_w2)
    x = x + _A_ref(_layernorm(x, axis=-1), A_wqkv, A_wo)
    x = x + _B_ref(_layernorm(x, axis=-1), B_w1, B_b1, B_w2)
    return x
```

```python
import math

import jax
import jax.numpy as jnp
import jax.experimental.pallas as pl
import jax.experimental.pallas.tpu as pltpu

_H = 32
_EPS = 1e-5
_TQ = 512
_TK = 128
_TR = 512
_TF = 256


def _layernorm(x):
    m = jnp.mean(x, axis=-1, keepdims=True)
    xc = x - m
    v = jnp.mean(xc * xc, axis=-1, keepdims=True)
    return xc * jax.lax.rsqrt(v + _EPS)


def _mish(h):
    sp = jnp.log1p(jnp.exp(-jnp.abs(h))) + jnp.where(h > 0, h, jnp.zeros_like(h))
    return h * jnp.tanh(sp)


def _fwd_kernel(x_ref, wqkv_ref, wo_ref, w1_ref, b1_ref, w2_ref, o_ref,
                xr_ref, wqt_ref, wvt_ref, k_ref, qt_ref, vt_ref, ot_ref,
                sa_ref, sb_ref, ma_ref, mb_ref):
    S, D = xr_ref.shape
    F = w1_ref.shape[1]
    DH = D // _H
    G = D // 128
    NQ = S // _TQ
    NU = _H * NQ
    NR = S // _TR
    qscale = (DH ** -0.5) * math.log2(math.e)
    bf16 = jnp.bfloat16
    f32 = jnp.float32

    xr_ref[...] = x_ref[...].astype(f32)
    wqt_ref[...] = wqkv_ref[:, 0:D].astype(f32).T.astype(bf16)
    wvt_ref[...] = wqkv_ref[:, 2 * D:3 * D].astype(f32).T.astype(bf16)

    nt_dims = (((1,), (1,)), ((), ()))
    tn_dims = (((0,), (0,)), ((), ()))

    def qkv_tile(r, carry):
        rows = pl.ds(pl.multiple_of(r * _TR, _TR), _TR)
        xn = _layernorm(xr_ref[rows, :]).astype(bf16)
        k = jnp.dot(xn, wqkv_ref[:, D:2 * D], preferred_element_type=f32).astype(bf16)
        for g in range(G):
            k_ref[g, rows, :] = k[:, g * 128:(g + 1) * 128]
        qt = jax.lax.dot_general(wqt_ref[...], xn, nt_dims, preferred_element_type=f32)
        qt_ref[:, rows] = (qt * qscale).astype(bf16)
        vt = jax.lax.dot_general(wvt_ref[...], xn, nt_dims, preferred_element_type=f32)
        vt_ref[:, rows] = vt.astype(bf16)
        return carry

    def unit_coords(u):
        h = u // NQ
        q0 = pl.multiple_of((u % NQ) * _TQ, _TQ)
        return h, q0

    def head_weights(u):
        h, q0 = unit_coords(u)
        g = h // (128 // DH)
        hh = h % (128 // DH)
        qt = qt_ref[pl.ds(pl.multiple_of(g * 128, 128), 128), pl.ds(q0, _TQ)]
        qi = pltpu.bitcast(qt, jnp.int32)
        prow = jax.lax.broadcasted_iota(jnp.int32, (64, _TQ), 0)
        w = jnp.where(prow // (DH // 2) == hh, qi, jnp.zeros_like(qi))
        return g, pltpu.bitcast(w, bf16)

    def attn_step(u1, s1_ref, m1_ref, u2, s2_ref, m2_ref):
        if u1 is not None:
            g, w = head_weights(u1)
            mrun = None
        if u2 is not None:
            h2, q2 = unit_coords(u2)
            d2 = pl.multiple_of(h2 * DH, DH)
            m2 = m2_ref[...]
            lrun = None
            acc = None
        for c in range(S // _TK):
            ks = pl.ds(c * _TK, _TK)
            if u1 is not None:
                s = jnp.dot(k_ref[g, ks, :], w, preferred_element_type=f32)
                s1_ref[ks, :] = s
                mc = jnp.max(s.reshape(_TK // 8, 8, _TQ), axis=0)
                mrun = mc if mrun is None else jnp.maximum(mrun, mc)
            if u2 is not None:
                p = jnp.exp2(s2_ref[ks, :] - m2)
                lc = jnp.sum(p.reshape(_TK // 8, 8, _TQ), axis=0)
                lrun = lc if lrun is None else lrun + lc
                a = jnp.dot(vt_ref[pl.ds(d2, DH), ks], p.astype(bf16),
                            preferred_element_type=f32)
                acc = a if acc is None else acc + a
        if u1 is not None:
            m1_ref[...] = jnp.max(mrun, axis=0, keepdims=True)
        if u2 is not None:
            l = jnp.sum(lrun, axis=0, keepdims=True)
            ot_ref[pl.ds(d2, DH), pl.ds(q2, _TQ)] = (acc / l).astype(bf16)

    def attn_pair(j, carry):
        u = 2 * j
        attn_step(u + 1, sb_ref, mb_ref, u, sa_ref, ma_ref)
        attn_step(u + 2, sa_ref, ma_ref, u + 1, sb_ref, mb_ref)
        return carry

    def dense_tile(r, carry):
        rows = pl.ds(pl.multiple_of(r * _TR, _TR), _TR)
        y = jax.lax.dot_general(ot_ref[:, rows], wo_ref[...], tn_dims,
                                preferred_element_type=f32)
        x = xr_ref[rows, :] + y
        xn = _layernorm(x).astype(bf16)
        acc = x
        for c in range(F // _TF):
            cs = pl.ds(c * _TF, _TF)
            h = jnp.dot(xn, w1_ref[:, cs], preferred_element_type=f32)
            h = h + b1_ref[:, cs].astype(f32)
            act = _mish(h).astype(bf16)
            acc = acc + jnp.dot(act, w2_ref[cs, :], preferred_element_type=f32)
        xr_ref[rows, :] = acc
        return carry

    def layer(i, carry):
        jax.lax.fori_loop(0, NR, qkv_tile, 0)
        attn_step(0, sa_ref, ma_ref, None, None, None)
        jax.lax.fori_loop(0, NU // 2 - 1, attn_pair, 0)
        attn_step(NU - 1, sb_ref, mb_ref, NU - 2, sa_ref, ma_ref)
        attn_step(None, None, None, NU - 1, sb_ref, mb_ref)
        jax.lax.fori_loop(0, NR, dense_tile, 0)
        return carry

    jax.lax.fori_loop(0, 2, layer, 0)
    o_ref[...] = xr_ref[...].astype(o_ref.dtype)


@jax.jit
def pallas_interleave_layers__mha_block__dense_activation_mish__prompt_kernel(
    A_x: jax.Array,
    A_wqkv: jax.Array,
    A_wo: jax.Array,
    B_x: jax.Array,
    B_w1: jax.Array,
    B_b1: jax.Array,
    B_w2: jax.Array,
):
    del B_x
    B, S, D = A_x.shape
    F = B_w1.shape[1]
    x = A_x.reshape(B * S, D)
    b1 = B_b1.reshape(1, F)
    f32, bf16 = jnp.float32, jnp.bfloat16
    scratch = [
        pltpu.VMEM((S, D), f32),
        pltpu.VMEM((D, D), bf16),
        pltpu.VMEM((D, D), bf16),
        pltpu.VMEM((D // 128, S, 128), bf16),
        pltpu.VMEM((D, S), bf16),
        pltpu.VMEM((D, S), bf16),
        pltpu.VMEM((D, S), bf16),
        pltpu.VMEM((S, _TQ), f32),
        pltpu.VMEM((S, _TQ), f32),
        pltpu.VMEM((1, _TQ), f32),
        pltpu.VMEM((1, _TQ), f32),
    ]
    out = pl.pallas_call(
        _fwd_kernel,
        out_shape=jax.ShapeDtypeStruct((B * S, D), A_x.dtype),
        scratch_shapes=scratch,
        compiler_params=pltpu.CompilerParams(vmem_limit_bytes=100 * 1024 * 1024),
    )(x, A_wqkv, A_wo, B_w1, b1, B_w2)
    return out.reshape(B, S, D)
```

```python
import math

import jax
import jax.numpy as jnp
import jax.experimental.pallas as pl
import jax.experimental.pallas.tpu as pltpu

_H = 32
_EPS = 1e-5
_TQ = 512
_TK = 128
_LAG = 1
_TOK = 3
_UNROLL = 4
_TR = 512
_TF = 256


def _layernorm(x):
    m = jnp.mean(x, axis=-1, keepdims=True)
    xc = x - m
    v = jnp.mean(xc * xc, axis=-1, keepdims=True)
    return xc * jax.lax.rsqrt(v + _EPS)


def _mish(h):
    sp = jnp.log1p(jnp.exp(-jnp.abs(h))) + jnp.where(h > 0, h, jnp.zeros_like(h))
    return h * jnp.tanh(sp)


def _fwd_kernel(x_ref, wqkv_ref, wo_ref, w1_ref, b1_ref, w2_ref, o_ref,
                xr_ref, wqt_ref, wvt_ref, k_ref, qt_ref, vt_ref, ot_ref,
                sa_ref, sb_ref, ma_ref, mb_ref, acc_ref, l_ref):
    S, D = xr_ref.shape
    F = w1_ref.shape[1]
    DH = D // _H
    G = D // 128
    NC = S // _TK
    NQ = S // _TQ
    NT = _TQ // 128
    NU = _H * NQ
    NR = S // _TR
    qscale = (DH ** -0.5) * math.log2(math.e)
    bf16 = jnp.bfloat16
    f32 = jnp.float32

    xr_ref[...] = x_ref[...].astype(f32)
    wqt_ref[...] = wqkv_ref[:, 0:D].astype(f32).T.astype(bf16)
    wvt_ref[...] = wqkv_ref[:, 2 * D:3 * D].astype(f32).T.astype(bf16)

    nt_dims = (((1,), (1,)), ((), ()))
    tn_dims = (((0,), (0,)), ((), ()))

    def qkv_tile(r, carry):
        rows = pl.ds(pl.multiple_of(r * _TR, _TR), _TR)
        xn = _layernorm(xr_ref[rows, :]).astype(bf16)
        k = jnp.dot(xn, wqkv_ref[:, D:2 * D], preferred_element_type=f32).astype(bf16)
        for g in range(G):
            k_ref[g, rows, :] = k[:, g * 128:(g + 1) * 128]
        qt = jax.lax.dot_general(wqt_ref[...], xn, nt_dims, preferred_element_type=f32)
        qt_ref[:, rows] = (qt * qscale).astype(bf16)
        vt = jax.lax.dot_general(wvt_ref[...], xn, nt_dims, preferred_element_type=f32)
        vt_ref[:, rows] = vt.astype(bf16)
        return carry

    def head_rows(u):
        return pl.multiple_of((u >> (NQ.bit_length() - 1)) * DH, DH)

    def query_cols(u):
        return pl.multiple_of((u & (NQ - 1)) * _TQ, _TQ)

    def head_weights(u):
        h = u >> (NQ.bit_length() - 1)
        g = h >> 3
        hh = h & 7
        qt = qt_ref[pl.ds(pl.multiple_of(g * 128, 128), 128), pl.ds(query_cols(u), _TQ)]
        qi = pltpu.bitcast(qt, jnp.int32)
        prow = jax.lax.broadcasted_iota(jnp.int32, (64, _TQ), 0)
        w = jnp.where((prow >> 3) == hh, qi, jnp.zeros_like(qi))
        return g, pltpu.bitcast(w, bf16)

    def scores(g, w, s_ref, c, mrun):
        ks = pl.ds(c * _TK, _TK)
        s = jnp.dot(k_ref[g, ks, :], w, preferred_element_type=f32)
        s_ref[ks, :] = s
        mc = jnp.max(s.reshape(_TK // 8, 8, _TQ), axis=0)
        return mc if mrun is None else jnp.maximum(mrun, mc)

    def exp_pv(d0, s_ref, m8, c, acc, lrun, hist):
        if len(hist) >= _TOK:
            z = jnp.minimum(jnp.maximum(hist[-_TOK][0:8, 0:128], 0.0), 0.0)
            m8 = m8 + jnp.concatenate([z] * NT, axis=1)
        ks = pl.ds(c * _TK, _TK)
        p = jnp.exp2(s_ref[ks, :].reshape(_TK // 8, 8, _TQ) - m8[None]).reshape(_TK, _TQ)
        lc = None
        for r8 in reversed(range(0, _TK, 8)):
            lc = p[r8:r8 + 8] if lc is None else lc + p[r8:r8 + 8]
        lrun = lc if lrun is None else lrun + lc
        a = jnp.dot(vt_ref[pl.ds(d0, DH), ks], p.astype(bf16), preferred_element_type=f32)
        acc = a if acc is None else acc + a
        hist.append(acc)
        return acc, lrun

    def finish(u, acc, lrun):
        l = jnp.sum(lrun, axis=0, keepdims=True)
        ot_ref[pl.ds(head_rows(u), DH), pl.ds(query_cols(u), _TQ)] = (acc / l).astype(bf16)

    def attn_step(u, sn_ref, mn_ref, sc_ref, mc_ref, state, do_q=True, extra=0):
        acc, lrun = state
        hist = []
        if do_q:
            g, w = head_weights(u + 1)
            mrun = None
        up = jnp.maximum(u - 1, 0)
        dp, dc = head_rows(up), head_rows(u)
        mp = jnp.broadcast_to(mn_ref[...], (8, _TQ))
        mcur = None
        for c in range(NC + extra):
            if do_q and c < NC:
                mrun = scores(g, w, sn_ref, c, mrun)
            if c < _LAG:
                acc, lrun = exp_pv(dp, sn_ref, mp, NC - _LAG + c, acc, lrun, hist)
                if c == _LAG - 1:
                    finish(up, acc, lrun)
                    acc = lrun = None
            else:
                if mcur is None:
                    mcur = jnp.broadcast_to(mc_ref[...], (8, _TQ))
                acc, lrun = exp_pv(dc, sc_ref, mcur, c - _LAG, acc, lrun, hist)
        if do_q:
            mn_ref[...] = jnp.max(mrun, axis=0, keepdims=True)
        return acc, lrun

    def attn_first():
        g, w = head_weights(0)
        mrun = None
        for c in range(NC):
            mrun = scores(g, w, sa_ref, c, mrun)
        ma_ref[...] = jnp.max(mrun, axis=0, keepdims=True)

    def attn_loop(j, carry):
        state = (acc_ref[...], l_ref[...])
        for t in range(0, _UNROLL, 2):
            u = _UNROLL * j + t
            state = attn_step(u, sb_ref, mb_ref, sa_ref, ma_ref, state)
            state = attn_step(u + 1, sa_ref, ma_ref, sb_ref, mb_ref, state)
        acc_ref[...] = state[0]
        l_ref[...] = state[1]
        return carry

    def attn_tail():
        state = (acc_ref[...], l_ref[...])
        n_loop = (NU - 2) // _UNROLL * _UNROLL
        for u in range(n_loop, NU - 2, 2):
            state = attn_step(jnp.int32(u), sb_ref, mb_ref, sa_ref, ma_ref, state)
            state = attn_step(jnp.int32(u + 1), sa_ref, ma_ref, sb_ref, mb_ref, state)
        state = attn_step(jnp.int32(NU - 2), sb_ref, mb_ref, sa_ref, ma_ref, state)
        acc, lrun = attn_step(jnp.int32(NU - 1), sa_ref, ma_ref, sb_ref, mb_ref, state,
                              do_q=False, extra=_LAG)
        finish(jnp.int32(NU - 1), acc, lrun)

    def dense_tile(r, carry):
        rows = pl.ds(pl.multiple_of(r * _TR, _TR), _TR)
        y = jax.lax.dot_general(ot_ref[:, rows], wo_ref[...], tn_dims,
                                preferred_element_type=f32)
        x = xr_ref[rows, :] + y
        xn = _layernorm(x).astype(bf16)
        acc = x
        for c in range(F // _TF):
            cs = pl.ds(c * _TF, _TF)
            h = jnp.dot(xn, w1_ref[:, cs], preferred_element_type=f32)
            h = h + b1_ref[:, cs].astype(f32)
            act = _mish(h).astype(bf16)
            acc = acc + jnp.dot(act, w2_ref[cs, :], preferred_element_type=f32)
        xr_ref[rows, :] = acc
        return carry

    sb_ref[pl.ds(S - _LAG * _TK, _LAG * _TK), :] = jnp.zeros((_LAG * _TK, _TQ), f32)
    mb_ref[...] = jnp.zeros_like(mb_ref)
    acc_ref[...] = jnp.ones_like(acc_ref)
    l_ref[...] = jnp.ones_like(l_ref)

    def layer(i, carry):
        jax.lax.fori_loop(0, NR, qkv_tile, 0)
        attn_first()
        jax.lax.fori_loop(0, (NU - 2) // _UNROLL, attn_loop, 0)
        attn_tail()
        jax.lax.fori_loop(0, NR, dense_tile, 0)
        return carry

    jax.lax.fori_loop(0, 2, layer, 0)
    o_ref[...] = xr_ref[...].astype(o_ref.dtype)


@jax.jit
def pallas_interleave_layers__mha_block__dense_activation_mish__prompt_kernel(
    A_x: jax.Array,
    A_wqkv: jax.Array,
    A_wo: jax.Array,
    B_x: jax.Array,
    B_w1: jax.Array,
    B_b1: jax.Array,
    B_w2: jax.Array,
):
    del B_x
    B, S, D = A_x.shape
    F = B_w1.shape[1]
    x = A_x.reshape(B * S, D)
    b1 = B_b1.reshape(1, F)
    f32, bf16 = jnp.float32, jnp.bfloat16
    scratch = [
        pltpu.VMEM((S, D), f32),
        pltpu.VMEM((D, D), bf16),
        pltpu.VMEM((D, D), bf16),
        pltpu.VMEM((D // 128, S, 128), bf16),
        pltpu.VMEM((D, S), bf16),
        pltpu.VMEM((D, S), bf16),
        pltpu.VMEM((D, S), bf16),
        pltpu.VMEM((S, _TQ), f32),
        pltpu.VMEM((S, _TQ), f32),
        pltpu.VMEM((1, _TQ), f32),
        pltpu.VMEM((1, _TQ), f32),
        pltpu.VMEM((D // _H, _TQ), f32),
        pltpu.VMEM((8, _TQ), f32),
    ]
    out = pl.pallas_call(
        _fwd_kernel,
        out_shape=jax.ShapeDtypeStruct((B * S, D), A_x.dtype),
        scratch_shapes=scratch,
        compiler_params=pltpu.CompilerParams(vmem_limit_bytes=100 * 1024 * 1024),
    )(x, A_wqkv, A_wo, B_w1, b1, B_w2)
    return out.reshape(B, S, D)
```

```python
import functools
import math

import jax
import jax.numpy as jnp
import jax.experimental.pallas as pl
import jax.experimental.pallas.tpu as pltpu

_H = 32
_EPS = 1e-5
_TQ = 512
_TK = 128
_LAG = 1
_TOK = 3
_UNROLL = 6
_TR = 256
_NS = 4
_TRQ = 128
_NSQ = 8
_TX = 512
_TF = 128


def _layernorm(x):
    m = jnp.mean(x, axis=-1, keepdims=True)
    xc = x - m
    v = jnp.mean(xc * xc, axis=-1, keepdims=True)
    return xc * jax.lax.rsqrt(v + _EPS)


def _mish(h):
    sp = jnp.log1p(jnp.exp(-jnp.abs(h))) + jnp.where(h > 0, h, jnp.zeros_like(h))
    return h * jnp.tanh(sp)


def _fwd_kernel(x_hbm, wqkv_hbm, wo_hbm, w1_hbm, b1_ref, w2_hbm, o_hbm,
                xo_ref, wqkv_ref, wo_ref, w1_ref, w2_ref, sem_x, sem_w, sem_o,
                xr_ref, wqt_ref, wvt_ref, k_ref, qt_ref, vt_ref, ot_ref,
                sa_ref, sb_ref, ma_ref, mb_ref, acc_ref, l_ref):
    S, D = xr_ref.shape
    F = w1_ref.shape[1]
    DH = D // _H
    G = D // 128
    NC = S // _TK
    NQ = S // _TQ
    NT = _TQ // 128
    NU = _H * NQ
    NX = S // _TX
    qscale = (DH ** -0.5) * math.log2(math.e)
    bf16 = jnp.bfloat16
    f32 = jnp.float32

    def tile_rows(r):
        return pl.ds(pl.multiple_of(r * _TX, _TX), _TX)

    def x_copy(r):
        return pltpu.make_async_copy(x_hbm.at[tile_rows(r)], xo_ref.at[tile_rows(r)], sem_x.at[r])

    def o_copy(r):
        rows = pl.ds(pl.multiple_of(r * _TR, _TR), _TR)
        return pltpu.make_async_copy(xo_ref.at[rows], o_hbm.at[rows], sem_o.at[r])

    w_copies = [pltpu.make_async_copy(src, dst, sem_w.at[n]) for n, (src, dst) in enumerate(
        [(wqkv_hbm, wqkv_ref), (wo_hbm, wo_ref), (w1_hbm, w1_ref), (w2_hbm, w2_ref)])]

    n_first = _NSQ * _TRQ // _TX
    w_copies[0].start()
    for r in range(n_first):
        x_copy(r).start()
    w_copies[0].wait()
    for r in range(n_first, NX):
        x_copy(r).start()
    for cp in w_copies[1:]:
        cp.start()

    wqt_ref[...] = wqkv_ref[:, 0:D].astype(f32).T.astype(bf16)
    wvt_ref[...] = wqkv_ref[:, 2 * D:3 * D].astype(f32).T.astype(bf16)

    nt_dims = (((1,), (1,)), ((), ()))
    tn_dims = (((0,), (0,)), ((), ()))

    def qkv_group(i, j):
        n_x = _NSQ * _TRQ // _TX

        @pl.when(i == 0)
        def _():
            for t in range(n_x):
                x_copy(j * n_x + t).wait()

        def ln1(t):
            rows = pl.ds(pl.multiple_of((j * _NSQ + t) * _TRQ, _TRQ), _TRQ)
            x = jnp.where(i == 0, xo_ref[rows, :].astype(f32), xr_ref[rows, :])
            xr_ref[rows, :] = x
            return _layernorm(x).astype(bf16)

        xn_next = ln1(0)
        for t in range(_NSQ):
            xn = xn_next
            if t + 1 < _NSQ:
                xn_next = ln1(t + 1)
            rows = pl.ds(pl.multiple_of((j * _NSQ + t) * _TRQ, _TRQ), _TRQ)
            k = jnp.dot(xn, wqkv_ref[:, D:2 * D], preferred_element_type=f32).astype(bf16)
            for g in range(G):
                k_ref[g, rows, :] = k[:, g * 128:(g + 1) * 128]
            qt = jax.lax.dot_general(wqt_ref[...], xn, nt_dims, preferred_element_type=f32)
            qt_ref[:, rows] = (qt * qscale).astype(bf16)
            vt = jax.lax.dot_general(wvt_ref[...], xn, nt_dims, preferred_element_type=f32)
            vt_ref[:, rows] = vt.astype(bf16)

    def head_rows(u):
        return pl.multiple_of((u >> (NQ.bit_length() - 1)) * DH, DH)

    def query_cols(u):
        return pl.multiple_of((u & (NQ - 1)) * _TQ, _TQ)

    def head_weights(u):
        h = u >> (NQ.bit_length() - 1)
        g = h >> 3
        hh = h & 7
        qt = qt_ref[pl.ds(pl.multiple_of(g * 128, 128), 128), pl.ds(query_cols(u), _TQ)]
        qi = pltpu.bitcast(qt, jnp.int32)
        prow = jax.lax.broadcasted_iota(jnp.int32, (64, _TQ), 0)
        w = jnp.where((prow >> 3) == hh, qi, jnp.zeros_like(qi))
        return g, pltpu.bitcast(w, bf16)

    def scores(g, w, s_ref, c, mrun):
        ks = pl.ds(c * _TK, _TK)
        s = jnp.dot(k_ref[g, ks, :], w, preferred_element_type=f32)
        s_ref[ks, :] = s
        mc = jnp.max(s.reshape(_TK // 8, 8, _TQ), axis=0)
        return mc if mrun is None else jnp.maximum(mrun, mc)

    def exp_pv(d0, s_ref, m8, c, acc, lrun, hist):
        if len(hist) >= _TOK:
            z = jnp.minimum(jnp.maximum(hist[-_TOK][0:8, 0:128], 0.0), 0.0)
            m8 = m8 + jnp.concatenate([z] * NT, axis=1)
        ks = pl.ds(c * _TK, _TK)
        p = jnp.exp2(s_ref[ks, :].reshape(_TK // 8, 8, _TQ) - m8[None]).reshape(_TK, _TQ)
        lc = None
        for r8 in reversed(range(0, _TK, 8)):
            lc = p[r8:r8 + 8] if lc is None else lc + p[r8:r8 + 8]
        lrun = lc if lrun is None else lrun + lc
        a = jnp.dot(vt_ref[pl.ds(d0, DH), ks], p.astype(bf16), preferred_element_type=f32)
        acc = a if acc is None else acc + a
        hist.append(acc)
        return acc, lrun

    def finish(u, acc, lrun):
        l = jnp.sum(lrun, axis=0, keepdims=True)
        ot_ref[pl.ds(head_rows(u), DH), pl.ds(query_cols(u), _TQ)] = (acc / l).astype(bf16)

    def attn_step(u, sn_ref, mn_ref, sc_ref, mc_ref, state, do_q=True, extra=0):
        acc, lrun = state
        hist = []
        if do_q:
            g, w = head_weights(u + 1)
            mrun = None
        up = jnp.maximum(u - 1, 0)
        dp, dc = head_rows(up), head_rows(u)
        mp = jnp.broadcast_to(mn_ref[...], (8, _TQ))
        mcur = None
        for c in range(NC + extra):
            if do_q and c < NC:
                mrun = scores(g, w, sn_ref, c, mrun)
            if c < _LAG:
                acc, lrun = exp_pv(dp, sn_ref, mp, NC - _LAG + c, acc, lrun, hist)
                if c == _LAG - 1:
                    finish(up, acc, lrun)
                    acc = lrun = None
            else:
                if mcur is None:
                    mcur = jnp.broadcast_to(mc_ref[...], (8, _TQ))
                acc, lrun = exp_pv(dc, sc_ref, mcur, c - _LAG, acc, lrun, hist)
        if do_q:
            mn_ref[...] = jnp.max(mrun, axis=0, keepdims=True)
        return acc, lrun

    def attn_first():
        g, w = head_weights(0)
        mrun = None
        for c in range(NC):
            mrun = scores(g, w, sa_ref, c, mrun)
        ma_ref[...] = jnp.max(mrun, axis=0, keepdims=True)

    def attn_loop(j, carry):
        state = (acc_ref[...], l_ref[...])
        for t in range(0, _UNROLL, 2):
            u = _UNROLL * j + t
            state = attn_step(u, sb_ref, mb_ref, sa_ref, ma_ref, state)
            state = attn_step(u + 1, sa_ref, ma_ref, sb_ref, mb_ref, state)
        acc_ref[...] = state[0]
        l_ref[...] = state[1]
        return carry

    def attn_tail():
        state = (acc_ref[...], l_ref[...])
        n_loop = (NU - 2) // _UNROLL * _UNROLL
        for u in range(n_loop, NU - 2, 2):
            state = attn_step(jnp.int32(u), sb_ref, mb_ref, sa_ref, ma_ref, state)
            state = attn_step(jnp.int32(u + 1), sa_ref, ma_ref, sb_ref, mb_ref, state)
        state = attn_step(jnp.int32(NU - 2), sb_ref, mb_ref, sa_ref, ma_ref, state)
        acc, lrun = attn_step(jnp.int32(NU - 1), sa_ref, ma_ref, sb_ref, mb_ref, state,
                              do_q=False, extra=_LAG)
        finish(jnp.int32(NU - 1), acc, lrun)

    def dense_group(i, j):
        def rows_of(t):
            return pl.ds(pl.multiple_of((j * _NS + t) * _TR, _TR), _TR)

        def proj_ln(t):
            rows = rows_of(t)
            y = jax.lax.dot_general(ot_ref[:, rows], wo_ref[...], tn_dims,
                                    preferred_element_type=f32)
            x = xr_ref[rows, :] + y
            return x, _layernorm(x).astype(bf16)

        nxt = proj_ln(0)
        for t in range(_NS):
            acc, xn = nxt
            if t + 1 < _NS:
                nxt = proj_ln(t + 1)
            for c in range(F // _TF):
                cs = pl.ds(c * _TF, _TF)
                h = jnp.dot(xn, w1_ref[:, cs], preferred_element_type=f32)
                h = h + b1_ref[cs].astype(f32)[None, :]
                act = _mish(h).astype(bf16)
                acc = acc + jnp.dot(act, w2_ref[cs, :], preferred_element_type=f32)
            xr_ref[rows_of(t), :] = acc
            xo_ref[rows_of(t), :] = acc.astype(bf16)
            o_copy(j * _NS + t).start()

    sb_ref[pl.ds(S - _LAG * _TK, _LAG * _TK), :] = jnp.zeros((_LAG * _TK, _TQ), f32)
    mb_ref[...] = jnp.zeros_like(mb_ref)
    acc_ref[...] = jnp.ones_like(acc_ref)
    l_ref[...] = jnp.ones_like(l_ref)

    def wait_copies(i):
        @pl.when(i == 0)
        def _():
            for cp in w_copies[1:]:
                cp.wait()

        @pl.when(i > 0)
        def _():
            for r in range(S // _TR):
                o_copy(r).wait()

    def layer(i, carry):
        pl.loop(0, S // (_NSQ * _TRQ))(functools.partial(qkv_group, i))
        attn_first()
        jax.lax.fori_loop(0, (NU - 2) // _UNROLL, attn_loop, 0)
        attn_tail()
        wait_copies(i)
        pl.loop(0, S // (_NS * _TR))(functools.partial(dense_group, i))
        return carry

    jax.lax.fori_loop(0, 2, layer, 0)
    for r in range(S // _TR):
        o_copy(r).wait()


@jax.jit
def pallas_interleave_layers__mha_block__dense_activation_mish__prompt_kernel(
    A_x: jax.Array,
    A_wqkv: jax.Array,
    A_wo: jax.Array,
    B_x: jax.Array,
    B_w1: jax.Array,
    B_b1: jax.Array,
    B_w2: jax.Array,
):
    del B_x
    B, S, D = A_x.shape
    F = B_w1.shape[1]
    x = A_x.reshape(B * S, D)
    f32, bf16 = jnp.float32, jnp.bfloat16
    scratch = [
        pltpu.VMEM((S, D), bf16),
        pltpu.VMEM(A_wqkv.shape, bf16),
        pltpu.VMEM(A_wo.shape, bf16),
        pltpu.VMEM(B_w1.shape, bf16),
        pltpu.VMEM(B_w2.shape, bf16),
        pltpu.SemaphoreType.DMA((S // _TX,)),
        pltpu.SemaphoreType.DMA((4,)),
        pltpu.SemaphoreType.DMA((S // _TR,)),
        pltpu.VMEM((S, D), f32),
        pltpu.VMEM((D, D), bf16),
        pltpu.VMEM((D, D), bf16),
        pltpu.VMEM((D // 128, S, 128), bf16),
        pltpu.VMEM((D, S), bf16),
        pltpu.VMEM((D, S), bf16),
        pltpu.VMEM((D, S), bf16),
        pltpu.VMEM((S, _TQ), f32),
        pltpu.VMEM((S, _TQ), f32),
        pltpu.VMEM((1, _TQ), f32),
        pltpu.VMEM((1, _TQ), f32),
        pltpu.VMEM((D // _H, _TQ), f32),
        pltpu.VMEM((8, _TQ), f32),
    ]
    hbm = pl.BlockSpec(memory_space=pl.ANY)
    out = pl.pallas_call(
        _fwd_kernel,
        out_shape=jax.ShapeDtypeStruct((B * S, D), A_x.dtype),
        in_specs=[hbm, hbm, hbm, hbm, pl.BlockSpec(memory_space=pltpu.VMEM), hbm],
        out_specs=hbm,
        scratch_shapes=scratch,
        compiler_params=pltpu.CompilerParams(vmem_limit_bytes=100 * 1024 * 1024),
    )(x, A_wqkv, A_wo, B_w1, B_b1, B_w2)
    return out.reshape(B, S, D)
```
